```python
import os as _os
_os.environ.setdefault("JAX_PLATFORMS", "cpu")
import jax
import jax.numpy as jnp

def _softmax(x, axis=-1):
    return jax.nn.softmax(x, axis=axis)
def _gelu(x):
    return jax.nn.gelu(x, approximate=True)
def _silu(x):
    return jax.nn.silu(x)
def _sigmoid(x):
    return jax.nn.sigmoid(x)
def _layernorm(x, axis=-1, eps=1e-5):
    m = jnp.mean(x, axis=axis, keepdims=True)
    v = jnp.var(x, axis=axis, keepdims=True)
    return (x - m) / jnp.sqrt(v + eps)
def _scatter_add(tgt, idx, src, axis=0):
    return tgt.at[idx].add(src)
def _segment_sum(src, seg, n):
    return jax.ops.segment_sum(src, seg, n)
class _Rng:
    def __init__(self, key):
        self._k = key
    def _next(self):
        self._k, sub = jax.random.split(self._k)
        return sub
    def normal(self, shape):
        return jax.random.normal(self._next(), shape, dtype=jnp.bfloat16)
    def randint(self, lo, hi, shape):
        return jax.random.randint(self._next(), shape, lo, hi, dtype=jnp.int32)
    def uniform(self, shape, lo=0.0, hi=1.0):
        return jax.random.uniform(self._next(), shape, jnp.bfloat16, lo, hi)
    def permutation(self, n):
        return jax.random.permutation(self._next(), n)


kernel_name = 'parallel_sum__softmax_full_mha__swiglu_ffn__prompt'

def setup_inputs():
    _rng = _Rng(jax.random.key(int.from_bytes(__import__("os").urandom(4), "little")))
    _w = (lambda a: (lambda t: t.astype(jnp.bfloat16) if jnp.issubdtype(t.dtype, jnp.floating) else t)(jnp.asarray(a)))
    def _A_setup():
        B, S, D = 1, 2048, 640
        return {
            "x": _w((lambda *s: _rng.normal(s) * 0.05)(B, S, D)),
            "wqkv": _w((lambda *s: _rng.normal(s) * 0.1)(D, 3 * D)),
            "wo": _w((lambda *s: _rng.normal(s) * 0.05)(D, D)),
        }
    _A_in = _A_setup()

    def _B_setup():
        B, S, D, F = 1, 2048, 640, 1536
        return {
            "x": _w((lambda *s: _rng.normal(s) * 0.05)(B, S, D)),
            "w_gate": _w((lambda *s: _rng.normal(s) * 0.05)(D, F)),
            "w_up": _w((lambda *s: _rng.normal(s) * 0.05)(D, F)),
            "w_down": _w((lambda *s: _rng.normal(s) * 0.05)(F, D)),
        }
    _B_in = _B_setup()

    return {
        "A_x": _A_in["x"],
        "A_wqkv": _A_in["wqkv"],
        "A_wo": _A_in["wo"],
        "B_x": _B_in["x"],
        "B_w_gate": _B_in["w_gate"],
        "B_w_up": _B_in["w_up"],
        "B_w_down": _B_in["w_down"],
    }

def reference(A_x, A_wqkv, A_wo, B_x, B_w_gate, B_w_up, B_w_down):
    def _A_ref(x, wqkv, wo):
        B, S, D = x.shape
        H = 32; Dh = D // H
        qkv = (lambda x, *d: x.transpose(*d))((x @ wqkv).reshape(B, S, 3, H, Dh), 2, 0, 3, 1, 4)
        q, k, v = qkv[0], qkv[1], qkv[2]
        scale = Dh ** -0.5
        scores = jnp.einsum("bhqd,bhkd->bhqk", q, k) * scale
        p = _softmax(scores, axis=-1)
        o = jnp.einsum("bhqk,bhkd->bhqd", p, v)
        return (lambda x, *d: x.transpose(*d))(o, 0, 2, 1, 3).reshape(B, S, D) @ wo

    def _B_ref(x, w_gate, w_up, w_down):
        g = _silu(x @ w_gate)
        u = x @ w_up
        return (g * u) @ w_down

    x = A_x
    xn = _layernorm(x, axis=-1)
    return x + _A_ref(xn, A_wqkv, A_wo) + _B_ref(xn, B_w_gate, B_w_up, B_w_down)
```

```python
import functools
import math

import jax
import jax.numpy as jnp
import jax.experimental.pallas as pl
import jax.experimental.pallas.tpu as pltpu

S = 2048
D = 640
H = 32
DH = 20
F = 1536
LANES = 128
HPT = 6
NT_QK = 6
TQ = 512
NQ = S // TQ
KC = 512
NKC = S // KC
RB = 512
NRB = S // RB
FC = 512
VROWS = 32
EPS = 1e-5
QSCALE = (DH ** -0.5) * math.log2(math.e)

_NT = (((1,), (1,)), ((), ()))


def _dot(a, b):
    return jnp.dot(a, b, preferred_element_type=jnp.float32)


def _dot_nt(a, b):
    return jax.lax.dot_general(a, b, _NT, preferred_element_type=jnp.float32)


def _kernel(x_ref, wqkv_ref, wo_ref, wg_ref, wu_ref, wd_ref, o_ref,
            xn_ref, q_ref, k_ref, vt_ref, wqk_ref, wvt_ref,
            s0_ref, s1_ref, m0_ref, ot_ref):
    step = pl.program_id(0)

    def masked_q(qblk, h):
        t = h // HPT
        off = (h % HPT) * DH
        q = q_ref[t, pl.ds(pl.multiple_of(qblk * TQ, TQ), TQ), :]
        lane = jax.lax.broadcasted_iota(jnp.int32, (TQ, LANES), 1)
        msk = jnp.logical_and(lane >= off, lane < off + DH)
        return jnp.where(msk, q, jnp.zeros_like(q)), t

    def qk_chunk(qm, t, c):
        return _dot_nt(k_ref[t, c * KC:(c + 1) * KC, :], qm)

    @pl.when(step == 0)
    def _prologue():
        for t in range(NT_QK):
            wqk_ref[:, t * LANES:(t + 1) * LANES] = (
                wqkv_ref[:, t * HPT * DH:t * HPT * DH + LANES])
            wqk_ref[:, (NT_QK + t) * LANES:(NT_QK + t + 1) * LANES] = (
                wqkv_ref[:, D + t * HPT * DH:D + t * HPT * DH + LANES])
        wvt_ref[...] = wqkv_ref[:, 2 * D:3 * D].T

        ones_blk = jnp.ones((VROWS - 24, RB), jnp.float32)

        def proj(r, carry):
            rows = pl.ds(pl.multiple_of(r * RB, RB), RB)
            x = x_ref[rows, :].astype(jnp.float32)
            mu = jnp.mean(x, axis=-1, keepdims=True)
            xc = x - mu
            var = jnp.mean(xc * xc, axis=-1, keepdims=True)
            xn = (xc * jax.lax.rsqrt(var + EPS)).astype(jnp.bfloat16)
            xn_ref[rows, :] = xn
            qk = _dot(xn, wqk_ref[...])
            for t in range(NT_QK):
                q_ref[t, rows, :] = (
                    qk[:, t * LANES:(t + 1) * LANES] * QSCALE).astype(jnp.bfloat16)
                k_ref[t, rows, :] = (
                    qk[:, (NT_QK + t) * LANES:(NT_QK + t + 1) * LANES]).astype(jnp.bfloat16)
            vt = _dot_nt(wvt_ref[...], xn)
            for h in range(H):
                a = (h * DH // 8) * 8
                blk = jnp.concatenate([vt[a:a + 24, :], ones_blk], axis=0)
                vt_ref[r, h] = blk.astype(jnp.bfloat16)
            return carry

        jax.lax.fori_loop(0, NRB, proj, 0)

        qm, t = masked_q(0, 0)
        m = None
        for c in range(NKC):
            s = qk_chunk(qm, t, c)
            s0_ref[c * KC:(c + 1) * KC, :] = s
            mc = jnp.max(s, axis=0, keepdims=True)
            m = mc if m is None else jnp.maximum(m, mc)
        m0_ref[...] = m

    def half(qm, t, dst_ref, src_ref, m_src, h_src):
        m_new = None
        acc = None
        for c in range(NKC):
            s = qk_chunk(qm, t, c)
            dst_ref[c * KC:(c + 1) * KC, :] = s
            mc = jnp.max(s, axis=0, keepdims=True)
            m_new = mc if m_new is None else jnp.maximum(m_new, mc)
            p = jnp.exp2(src_ref[c * KC:(c + 1) * KC, :] - m_src).astype(jnp.bfloat16)
            pv = _dot(vt_ref[c, h_src], p)
            acc = pv if acc is None else acc + pv
        return m_new, acc

    def pair(j, carry):
        ha = 2 * j
        hb = ha + 1
        last = j == H // 2 - 1
        hn = jnp.where(last, 0, ha + 2)
        qn = jnp.where(last, jnp.minimum(step + 1, NQ - 1), step)

        qm_b, t_b = masked_q(step, hb)
        m1, acc_a = half(qm_b, t_b, s1_ref, s0_ref, m0_ref[...], ha)
        qm_n, t_n = masked_q(qn, hn)
        m0, acc_b = half(qm_n, t_n, s0_ref, s1_ref, m1, hb)
        m0_ref[...] = m0

        oa = acc_a[0:24, :] / acc_a[24:25, :]
        ob = acc_b[0:24, :] / acc_b[24:25, :]
        sub = jax.lax.broadcasted_iota(jnp.int32, (8, TQ), 0)
        mid = jnp.where(sub < 4, oa[16:24, :], ob[0:8, :])
        blk = jnp.concatenate([oa[0:16, :], mid, ob[8:24, :]], axis=0)
        ot_ref[pl.ds(pl.multiple_of(j * 2 * DH, 8), 2 * DH), :] = blk
        return carry

    jax.lax.fori_loop(0, H // 2, pair, 0)

    rows = pl.ds(pl.multiple_of(step * TQ, TQ), TQ)
    o = ot_ref[...].T.astype(jnp.bfloat16)
    acc = x_ref[rows, :].astype(jnp.float32) + _dot(o, wo_ref[...])
    xn = xn_ref[rows, :]
    for f in range(F // FC):
        g = _dot(xn, wg_ref[:, f * FC:(f + 1) * FC])
        u = _dot(xn, wu_ref[:, f * FC:(f + 1) * FC])
        hmid = (g * jax.nn.sigmoid(g) * u).astype(jnp.bfloat16)
        acc = acc + _dot(hmid, wd_ref[f * FC:(f + 1) * FC, :])
    o_ref[...] = acc.astype(o_ref.dtype)


@jax.jit
def pallas_parallel_sum__softmax_full_mha__swiglu_ffn__prompt_kernel(
    A_x: jax.Array,
    A_wqkv: jax.Array,
    A_wo: jax.Array,
    B_x: jax.Array,
    B_w_gate: jax.Array,
    B_w_up: jax.Array,
    B_w_down: jax.Array,
):
    del B_x
    assert RB == KC
    x = A_x.reshape(S, D)
    full = lambda shape: pl.BlockSpec(shape, lambda i: (0,) * len(shape))
    out = pl.pallas_call(
        _kernel,
        grid=(NQ,),
        in_specs=[
            full((S, D)),
            full((D, 3 * D)),
            full((D, D)),
            full((D, F)),
            full((D, F)),
            full((F, D)),
        ],
        out_specs=pl.BlockSpec((TQ, D), lambda i: (i, 0)),
        out_shape=jax.ShapeDtypeStruct((S, D), A_x.dtype),
        scratch_shapes=[
            pltpu.VMEM((S, D), jnp.bfloat16),
            pltpu.VMEM((NT_QK, S, LANES), jnp.bfloat16),
            pltpu.VMEM((NT_QK, S, LANES), jnp.bfloat16),
            pltpu.VMEM((NRB, H, VROWS, RB), jnp.bfloat16),
            pltpu.VMEM((D, 2 * NT_QK * LANES), jnp.bfloat16),
            pltpu.VMEM((D, D), jnp.bfloat16),
            pltpu.VMEM((S, TQ), jnp.float32),
            pltpu.VMEM((S, TQ), jnp.float32),
            pltpu.VMEM((1, TQ), jnp.float32),
            pltpu.VMEM((D, TQ), jnp.float32),
        ],
        compiler_params=pltpu.CompilerParams(
            dimension_semantics=("arbitrary",),
            vmem_limit_bytes=100 * 1024 * 1024,
        ),
    )(x, A_wqkv, A_wo, B_w_gate, B_w_up, B_w_down)
    return out.reshape(A_x.shape)
```

```python
import math

import jax
import jax.numpy as jnp
import jax.experimental.pallas as pl
import jax.experimental.pallas.tpu as pltpu

S = 2048
D = 640
H = 32
DH = 20
F = 1536
LANES = 128
NT_K = 6
TQ = 512
NQ = S // TQ
KC = 128
NKC = S // KC
RB = 512
NRB = S // RB
FC = 512
PB = 256
VROWS = 24
NH = 8
SKEW = 2
NBUF = 4
EPS = 1e-5
QSCALE = (DH ** -0.5) * math.log2(math.e)
STRADDLE = tuple(h for h in range(H) if (h * DH) % LANES > LANES - DH)
XOFF = tuple(24 * i + 4 * (i >= 2) for i in range(len(STRADDLE)))

_NN = (((1,), (0,)), ((), ()))
_NT = (((1,), (1,)), ((), ()))


def _dot(a, b):
    return jax.lax.dot_general(a, b, _NN, preferred_element_type=jnp.float32)


def _dot_nt(a, b):
    return jax.lax.dot_general(a, b, _NT, preferred_element_type=jnp.float32)


def _kernel(x_hbm, wqkv_hbm, wo_hbm, wg_hbm, wu_hbm, wd_hbm, o_ref,
            x_ref, wqkv_ref, wo_ref, wg_ref, wu_ref, wd_ref, sems,
            xn_ref, qt_ref, k_ref, vt_ref, wkx_ref, wqvt_ref, m0_ref, ot_ref, *s_refs):
    step = pl.program_id(0)

    def x_copy(r):
        rows = pl.ds(r * RB, RB)
        return pltpu.make_async_copy(x_hbm.at[rows, :], x_ref.at[rows, :], sems.at[r])

    def wqkv_copy(i):
        cols = pl.ds(i * D, D)
        return pltpu.make_async_copy(wqkv_hbm.at[:, cols], wqkv_ref.at[:, cols], sems.at[NRB + i])

    def w_copy(i):
        src, dst = ((wg_hbm, wg_ref), (wu_hbm, wu_ref), (wd_hbm, wd_ref), (wo_hbm, wo_ref))[i]
        return pltpu.make_async_copy(src, dst, sems.at[NRB + 3 + i])

    def head_q(qblk, h):
        col = h * DH
        t = col >> 7
        off = col & (LANES - 1)
        cross = off > LANES - DH
        off = jnp.where(cross, 24 * t + jnp.where(t >= 2, 4, 0), off)
        t = jnp.where(cross, NT_K - 1, t)
        base = pl.multiple_of(col - off, 8)
        q = qt_ref[qblk, pl.ds(base, LANES), :]
        row = jax.lax.broadcasted_iota(jnp.int32, (LANES, TQ), 0)
        msk = jnp.logical_and(row >= off, row < off + DH)
        return jnp.where(msk, q, 0.0).astype(jnp.bfloat16), t

    def qk_chunk(qm, t, dst_ref, c):
        s = _dot(k_ref[t, c * KC:(c + 1) * KC, :], qm)
        dst_ref[c * KC:(c + 1) * KC, :] = s
        return jnp.max(s.reshape(KC // 8, 8, TQ), axis=0)

    def layernorm(r):
        rows = slice(r * RB, (r + 1) * RB)
        x = x_ref[rows, :].astype(jnp.float32)
        mu = jnp.mean(x, axis=-1, keepdims=True)
        xc = x - mu
        var = jnp.mean(xc * xc, axis=-1, keepdims=True)
        xn_ref[rows, :] = (xc * jax.lax.rsqrt(var + EPS)).astype(jnp.bfloat16)

    def k_proj(r):
        rows = slice(r * RB, (r + 1) * RB)
        kk = _dot(xn_ref[rows, :], wqkv_ref[:, D:D + 4 * LANES])
        for t in range(4):
            k_ref[t, rows, :] = kk[:, t * LANES:(t + 1) * LANES].astype(jnp.bfloat16)

    def kx_proj(r):
        for i in range(2):
            rows = slice(r * RB + i * RB // 2, r * RB + (i + 1) * RB // 2)
            kk = _dot(xn_ref[rows, :], wkx_ref[...])
            for t in range(2):
                k_ref[4 + t, rows, :] = kk[:, t * LANES:(t + 1) * LANES].astype(jnp.bfloat16)

    @pl.when(step == 0)
    def _prologue():
        x_copy(0).start()
        wqkv_copy(1).start()
        x_copy(1).start()
        x_copy(2).start()
        x_copy(3).start()
        wqkv_copy(0).start()
        wqkv_copy(2).start()

        x_copy(0).wait()
        layernorm(0)
        wqkv_copy(1).wait()
        k_proj(0)
        lane = jax.lax.broadcasted_iota(jnp.int32, (D, LANES), 1)
        wkx = None
        for h, o in zip(STRADDLE, XOFF):
            c0 = D + h * DH - o
            win = wqkv_ref[:, c0:c0 + LANES]
            wkx = win if wkx is None else jnp.where(lane >= o, win, wkx)
        wkx_ref[:, 0:LANES] = wqkv_ref[:, D + 4 * LANES:2 * D]
        wkx_ref[:, LANES:2 * LANES] = wkx

        x_copy(1).wait()
        x_copy(2).wait()
        kx_proj(0)
        layernorm(1)
        k_proj(1)
        kx_proj(1)
        layernorm(2)
        k_proj(2)

        x_copy(3).wait()
        wqkv_copy(0).wait()
        wqkv_copy(2).wait()
        for i in range(4):
            w_copy(i).start()
        kx_proj(2)
        layernorm(3)
        k_proj(3)
        kx_proj(3)
        wqvt_ref[0:D, :] = wqkv_ref[:, 0:D].T
        wqvt_ref[D:2 * D, :] = wqkv_ref[:, 2 * D:3 * D].T

        sub = jax.lax.broadcasted_iota(jnp.int32, (8, RB), 0)

        def qv_proj(r, carry):
            rows = pl.ds(pl.multiple_of(r * RB, RB), RB)
            qv = _dot_nt(wqvt_ref[...], xn_ref[rows, :])
            qt_ref[r] = qv[0:D, :] * QSCALE
            for h in range(H):
                a = D + (h * DH // 8) * 8
                if h % 2 == 0:
                    vt_ref[r, h, 0:16, :] = qv[a:a + 16, :]
                    vt_ref[r, h, 16:24, :] = jnp.where(sub == 4, 1.0, qv[a + 16:a + 24, :])
                else:
                    vt_ref[r, h, 0:8, :] = jnp.where(sub == 0, 1.0, qv[a:a + 8, :])
                    vt_ref[r, h, 8:24, :] = qv[a + 8:a + 24, :]
            return carry

        jax.lax.fori_loop(0, NRB, qv_proj, 0)

        qm, t = head_q(0, 0)
        m = None
        for c in range(NKC):
            mc = qk_chunk(qm, t, s_refs[0], c)
            m = mc if m is None else jnp.maximum(m, mc)
        m0_ref[...] = jnp.max(m, axis=0, keepdims=True)
        for i in range(4):
            w_copy(i).wait()

    def group(j, carry):
        h0 = NH * j
        last = j == H // NH - 1
        zero = pl.multiple_of((step // NQ) * 8, 8)

        nxt = [(step, h0 + p + 1) for p in range(NH - 1)]
        nxt.append((jnp.where(last, jnp.minimum(step + 1, NQ - 1), step),
                    jnp.where(last, 0, h0 + NH)))

        m = [None] * (NH + 1)
        m[0] = m0_ref[...]
        acc = [None] * NH
        qm_cur = [None] * NH

        def do_qk(g):
            p, c = divmod(g, NKC)
            if c == 0:
                qm_cur[p] = head_q(*nxt[p])
            qm, t = qm_cur[p]
            mc = qk_chunk(qm, t, s_refs[(p + 1) % NBUF], c)
            m[p + 1] = mc if m[p + 1] is None else jnp.maximum(m[p + 1], mc)
            if c == NKC - 1:
                m[p + 1] = jnp.max(m[p + 1], axis=0, keepdims=True)

        def do_pv(g):
            p, c = divmod(g, NKC)
            src = s_refs[p % NBUF]
            if p > 0:
                s = src[pl.ds(zero + c * KC, KC), :]
            else:
                s = src[c * KC:(c + 1) * KC, :]
            pr = jnp.exp2(s - m[p]).astype(jnp.bfloat16)
            off = (c * KC) % RB
            pv = _dot(vt_ref[(c * KC) // RB, h0 + p, :, off:off + KC], pr)
            acc[p] = pv if acc[p] is None else acc[p] + pv
            if c == NKC - 1 and p % 2 == 1:
                acc_a, acc_b = acc[p - 1], acc[p]
                oa = acc_a / acc_a[DH:DH + 1, :]
                ob = acc_b / acc_b[0:1, :]
                sub = jax.lax.broadcasted_iota(jnp.int32, (8, TQ), 0)
                mid = jnp.where(sub < 4, oa[16:24, :], ob[0:8, :])
                blk = jnp.concatenate([oa[0:16, :], mid, ob[8:24, :]], axis=0)
                row = pl.multiple_of((h0 + p - 1) * DH, 8)
                ot_ref[pl.ds(row, 2 * DH), :] = blk

        total = NH * NKC
        for g in range(total + SKEW):
            if g < total:
                do_qk(g)
            if g >= SKEW:
                do_pv(g - SKEW)
        m0_ref[...] = m[NH]
        return carry

    jax.lax.fori_loop(0, H // NH, group, 0)

    def epilogue(i, carry):
        cols = pl.ds(pl.multiple_of(i * PB, PB), PB)
        rows = pl.ds(pl.multiple_of(step * TQ + i * PB, PB), PB)
        xn = xn_ref[rows, :]
        acc = x_ref[rows, :].astype(jnp.float32)
        for f in range(F // FC):
            g = _dot(xn, wg_ref[:, f * FC:(f + 1) * FC])
            u = _dot(xn, wu_ref[:, f * FC:(f + 1) * FC])
            hmid = (g * jax.nn.sigmoid(g) * u).astype(jnp.bfloat16)
            acc = acc + _dot(hmid, wd_ref[f * FC:(f + 1) * FC, :])
            if f == 0:
                o = ot_ref[:, cols].T.astype(jnp.bfloat16)
                acc = acc + _dot(o, wo_ref[...])
        o_ref[cols, :] = acc.astype(o_ref.dtype)
        return carry

    jax.lax.fori_loop(0, TQ // PB, epilogue, 0)


@jax.jit
def pallas_parallel_sum__softmax_full_mha__swiglu_ffn__prompt_kernel(
    A_x: jax.Array,
    A_wqkv: jax.Array,
    A_wo: jax.Array,
    B_x: jax.Array,
    B_w_gate: jax.Array,
    B_w_up: jax.Array,
    B_w_down: jax.Array,
):
    del B_x
    assert A_x.shape == (1, S, D) and TQ == RB
    bf16 = jnp.bfloat16
    f32 = jnp.float32
    out = pl.pallas_call(
        _kernel,
        grid=(NQ,),
        in_specs=[pl.BlockSpec(memory_space=pl.ANY)] * 6,
        out_specs=pl.BlockSpec((TQ, D), lambda i: (i, 0)),
        out_shape=jax.ShapeDtypeStruct((S, D), A_x.dtype),
        scratch_shapes=[
            pltpu.VMEM((S, D), bf16),
            pltpu.VMEM((D, 3 * D), bf16),
            pltpu.VMEM((D, D), bf16),
            pltpu.VMEM((D, F), bf16),
            pltpu.VMEM((D, F), bf16),
            pltpu.VMEM((F, D), bf16),
            pltpu.SemaphoreType.DMA((NRB + 7,)),
            pltpu.VMEM((S, D), bf16),
            pltpu.VMEM((NQ, D, TQ), f32),
            pltpu.VMEM((NT_K, S, LANES), bf16),
            pltpu.VMEM((NRB, H, VROWS, RB), f32),
            pltpu.VMEM((D, 2 * LANES), bf16),
            pltpu.VMEM((2 * D, D), bf16),
            pltpu.VMEM((1, TQ), f32),
            pltpu.VMEM((D, TQ), f32),
        ] + [pltpu.VMEM((S, TQ), f32) for _ in range(NBUF)],
        compiler_params=pltpu.CompilerParams(
            dimension_semantics=("arbitrary",),
            vmem_limit_bytes=110 * 1024 * 1024,
        ),
    )(A_x.reshape(S, D), A_wqkv, A_wo, B_w_gate, B_w_up, B_w_down)
    return out.reshape(A_x.shape)
```

```python
import math

import jax
import jax.numpy as jnp
import jax.experimental.pallas as pl
import jax.experimental.pallas.tpu as pltpu

S = 2048
D = 640
H = 32
DH = 20
F = 1536
LANES = 128
NT_K = 6
TQ = 512
NQ = S // TQ
KC = 128
NKC = S // KC
RB = 512
NRB = S // RB
FC = 512
VROWS = 24
NH = 8
FB = TQ // (H // NH)
SKEW = 1
NBUF = 4
OB = 128
ZSPLIT = 20
EPS = 1e-5
QSCALE = (DH ** -0.5) * math.log2(math.e)
STRADDLE = tuple(h for h in range(H) if (h * DH) % LANES > LANES - DH)
XOFF = tuple(24 * i + 4 * (i >= 2) for i in range(len(STRADDLE)))

_NN = (((1,), (0,)), ((), ()))
_NT = (((1,), (1,)), ((), ()))


def _dot(a, b):
    return jax.lax.dot_general(a, b, _NN, preferred_element_type=jnp.float32)


def _dot_nt(a, b):
    return jax.lax.dot_general(a, b, _NT, preferred_element_type=jnp.float32)


def _q_window(h):
    off = XOFF[STRADDLE.index(h)] if h in STRADDLE else (h * DH) % LANES
    return h * DH - off, off


def _kernel(x_hbm, wqkv_hbm, wo_hbm, wg_hbm, wu_hbm, wd_hbm, o_hbm,
            x_ref, wqkv_ref, wo_ref, wg_ref, wu_ref, wd_ref, sems,
            xn_ref, qt_ref, k_ref, vt_ref, wkx_ref, wqvt_ref, y_ref, ot_ref,
            o_ref, osems, *s_refs):
    step = pl.program_id(0)

    def x_copy(r):
        rows = pl.ds(r * RB, RB)
        return pltpu.make_async_copy(x_hbm.at[rows, :], x_ref.at[rows, :], sems.at[r])

    def wqkv_copy(i):
        cols = pl.ds(i * D, D)
        return pltpu.make_async_copy(wqkv_hbm.at[:, cols], wqkv_ref.at[:, cols], sems.at[NRB + i])

    def w_copy(i):
        src, dst = ((wg_hbm, wg_ref), (wu_hbm, wu_ref), (wd_hbm, wd_ref), (wo_hbm, wo_ref))[i]
        return pltpu.make_async_copy(src, dst, sems.at[NRB + 3 + i])

    def o_copy(blk, i):
        dst = pl.ds(pl.multiple_of(blk * TQ + i * OB, OB), OB)
        return pltpu.make_async_copy(o_ref.at[pl.ds(i * OB, OB), :], o_hbm.at[dst, :], osems.at[i])

    def layernorm(r):
        rows = slice(r * RB, (r + 1) * RB)
        x = x_ref[rows, :].astype(jnp.float32)
        mu = jnp.mean(x, axis=-1, keepdims=True)
        xc = x - mu
        var = jnp.mean(xc * xc, axis=-1, keepdims=True)
        xn_ref[rows, :] = (xc * jax.lax.rsqrt(var + EPS)).astype(jnp.bfloat16)

    def k_proj(r):
        rows = slice(r * RB, (r + 1) * RB)
        kk = _dot(xn_ref[rows, :], wqkv_ref[:, D:D + 4 * LANES])
        for t in range(4):
            k_ref[t, rows, :] = kk[:, t * LANES:(t + 1) * LANES].astype(jnp.bfloat16)

    def kx_proj(r):
        for i in range(2):
            rows = slice(r * RB + i * RB // 2, r * RB + (i + 1) * RB // 2)
            kk = _dot(xn_ref[rows, :], wkx_ref[...])
            for t in range(2):
                k_ref[4 + t, rows, :] = kk[:, t * LANES:(t + 1) * LANES].astype(jnp.bfloat16)

    def zero_fill(h_lo, h_hi):
        for h in range(h_lo, h_hi):
            _, off = _q_window(h)
            a, b = 8 * (off // 16), 8 * ((off + DH - 1) // 16 + 1)
            if a > 0:
                qt_ref[:, h, 0:a, :] = jnp.zeros((NQ, a, TQ), jnp.uint32)
            if b < LANES // 2:
                qt_ref[:, h, b:LANES // 2, :] = jnp.zeros((NQ, LANES // 2 - b, TQ), jnp.uint32)

    @pl.when(step == 0)
    def _prologue():
        x_copy(0).start()
        wqkv_copy(1).start()
        x_copy(1).start()
        x_copy(2).start()
        x_copy(3).start()
        wqkv_copy(0).start()
        wqkv_copy(2).start()

        zero_fill(0, ZSPLIT)
        x_copy(0).wait()
        layernorm(0)
        zero_fill(ZSPLIT, H)
        wqkv_copy(1).wait()
        k_proj(0)
        lane = jax.lax.broadcasted_iota(jnp.int32, (D, LANES), 1)
        wkx = None
        for h, o in zip(STRADDLE, XOFF):
            c0 = D + h * DH - o
            win = wqkv_ref[:, c0:c0 + LANES]
            wkx = win if wkx is None else jnp.where(lane >= o, win, wkx)
        wkx_ref[:, 0:LANES] = wqkv_ref[:, D + 4 * LANES:2 * D]
        wkx_ref[:, LANES:2 * LANES] = wkx

        x_copy(1).wait()
        x_copy(2).wait()
        kx_proj(0)
        layernorm(1)
        k_proj(1)
        kx_proj(1)
        layernorm(2)
        k_proj(2)

        x_copy(3).wait()
        wqkv_copy(0).wait()
        wqkv_copy(2).wait()
        for i in range(4):
            w_copy(i).start()
        kx_proj(2)
        layernorm(3)
        k_proj(3)
        kx_proj(3)
        wqvt_ref[0:D, :] = wqkv_ref[:, 0:D].T
        wqvt_ref[D:2 * D, :] = wqkv_ref[:, 2 * D:3 * D].T

        sub = jax.lax.broadcasted_iota(jnp.int32, (8, RB), 0)
        row16 = jax.lax.broadcasted_iota(jnp.int32, (16, RB), 0)

        def qv_proj(r, carry):
            rows = pl.ds(pl.multiple_of(r * RB, RB), RB)
            qv = _dot_nt(wqvt_ref[...], xn_ref[rows, :])
            qs = qv[0:D, :] * QSCALE
            for h in range(H):
                base, off = _q_window(h)
                for i in range(off // 16, (off + DH - 1) // 16 + 1):
                    lo, hi = off - 16 * i, off + DH - 16 * i
                    blk = qs[base + 16 * i:base + 16 * (i + 1), :]
                    if lo > 0 or hi < 16:
                        blk = jnp.where(jnp.logical_and(row16 >= lo, row16 < hi), blk, 0.0)
                    qt_ref[r, h, 8 * i:8 * (i + 1), :] = pltpu.bitcast(
                        blk.astype(jnp.bfloat16), jnp.uint32)
            for h in range(H):
                a = D + (h * DH // 8) * 8
                if h % 2 == 0:
                    vt_ref[r, h, 0:16, :] = qv[a:a + 16, :]
                    vt_ref[r, h, 16:24, :] = jnp.where(sub == 4, 1.0, qv[a + 16:a + 24, :])
                else:
                    vt_ref[r, h, 0:8, :] = jnp.where(sub == 0, 1.0, qv[a:a + 8, :])
                    vt_ref[r, h, 8:24, :] = qv[a + 8:a + 24, :]
            return carry

        jax.lax.fori_loop(0, NRB, qv_proj, 0)
        for i in range(4):
            w_copy(i).wait()

    def group(j, carry):
        h0 = NH * j
        zero = pl.multiple_of((step // NQ) * 8, 8)

        m = [None] * NH
        acc = [None] * NH

        def do_qk(g):
            p, c = divmod(g, NKC)
            col = (h0 + p) * DH
            t = jnp.where((col & (LANES - 1)) > LANES - DH, NT_K - 1, col >> 7)
            qm = pltpu.bitcast(qt_ref[step, h0 + p], jnp.bfloat16)
            s = _dot(k_ref[t, c * KC:(c + 1) * KC, :], qm)
            s_refs[p % NBUF][c * KC:(c + 1) * KC, :] = s
            mc = jnp.max(s.reshape(KC // 8, 8, TQ), axis=0)
            m[p] = mc if m[p] is None else jnp.maximum(m[p], mc)
            if c == NKC - 1:
                m[p] = jnp.max(m[p], axis=0, keepdims=True)

        def do_pv(g):
            p, c = divmod(g, NKC)
            s = s_refs[p % NBUF][pl.ds(zero + c * KC, KC), :]
            pr = jnp.exp2(s - m[p]).astype(jnp.bfloat16)
            off = (c * KC) % RB
            pv = _dot(vt_ref[(c * KC) // RB, h0 + p, :, off:off + KC], pr)
            acc[p] = pv if acc[p] is None else acc[p] + pv
            if c == NKC - 1 and p % 2 == 1:
                acc_a, acc_b = acc[p - 1], acc[p]
                oa = acc_a / acc_a[DH:DH + 1, :]
                ob = acc_b / acc_b[0:1, :]
                sub = jax.lax.broadcasted_iota(jnp.int32, (8, TQ), 0)
                mid = jnp.where(sub < 4, oa[16:24, :], ob[0:8, :])
                blk = jnp.concatenate([oa[0:16, :], mid, ob[8:24, :]], axis=0)
                row = pl.multiple_of((h0 + p - 1) * DH, 8)
                ot_ref[pl.ds(row, 2 * DH), :] = blk

        rows = pl.ds(pl.multiple_of(step * TQ + j * FB, FB), FB)
        st = {}

        def up_piece(name, w_ref, f, k):
            part = _dot(xn_ref[rows, k * LANES:(k + 1) * LANES],
                        w_ref[k * LANES:(k + 1) * LANES, f * FC:(f + 1) * FC])
            st[name, f] = part if k == 0 else st[name, f] + part

        def down_piece(f):
            g, u = st["g", f], st["u", f]
            sig = 0.5 * jnp.tanh(0.5 * g) + 0.5
            hmid = (g * sig * u).astype(jnp.bfloat16)
            part = _dot(hmid, wd_ref[f * FC:(f + 1) * FC, :])
            st["y"] = (x_ref[rows, :].astype(jnp.float32) if f == 0 else st["y"]) + part

        ffn = []
        for f in range(F // FC):
            ffn += [(up_piece, "g", wg_ref, f, k) for k in range(D // LANES)]
            ffn += [(up_piece, "u", wu_ref, f, k) for k in range(D // LANES)]
            if f >= 1:
                ffn.append((down_piece, f - 1))
        ffn.append((down_piece, F // FC - 1))

        total = NH * NKC
        lag = NKC + SKEW
        for g in range(total):
            do_qk(g)
            if g >= lag:
                do_pv(g - lag)
        used = 0
        for i in range(lag):
            while used < (3 * (i + 1)) // 2:
                ffn[used][0](*ffn[used][1:])
                used += 1
            do_pv(total - lag + i)
        for piece in ffn[used:]:
            piece[0](*piece[1:])
        y_ref[pl.ds(pl.multiple_of(j * FB, FB), FB), :] = st["y"]
        return carry

    jax.lax.fori_loop(0, H // NH, group, 0)

    @pl.when(step > 0)
    def _():
        for i in range(TQ // OB):
            o_copy(step - 1, i).wait()

    for i in range(TQ // OB):
        cols = slice(i * OB, (i + 1) * OB)
        o = ot_ref[:, cols].T.astype(jnp.bfloat16)
        o_ref[cols, :] = (y_ref[cols, :] + _dot(o, wo_ref[...])).astype(o_ref.dtype)
        o_copy(step, i).start()

    @pl.when(step == NQ - 1)
    def _():
        for i in range(TQ // OB):
            o_copy(step, i).wait()


@jax.jit
def pallas_parallel_sum__softmax_full_mha__swiglu_ffn__prompt_kernel(
    A_x: jax.Array,
    A_wqkv: jax.Array,
    A_wo: jax.Array,
    B_x: jax.Array,
    B_w_gate: jax.Array,
    B_w_up: jax.Array,
    B_w_down: jax.Array,
):
    del B_x
    assert A_x.shape == (1, S, D) and TQ == RB
    bf16 = jnp.bfloat16
    f32 = jnp.float32
    out = pl.pallas_call(
        _kernel,
        grid=(NQ,),
        in_specs=[pl.BlockSpec(memory_space=pl.ANY)] * 6,
        out_specs=pl.BlockSpec(memory_space=pl.ANY),
        out_shape=jax.ShapeDtypeStruct((S, D), A_x.dtype),
        scratch_shapes=[
            pltpu.VMEM((S, D), bf16),
            pltpu.VMEM((D, 3 * D), bf16),
            pltpu.VMEM((D, D), bf16),
            pltpu.VMEM((D, F), bf16),
            pltpu.VMEM((D, F), bf16),
            pltpu.VMEM((F, D), bf16),
            pltpu.SemaphoreType.DMA((NRB + 7,)),
            pltpu.VMEM((S, D), bf16),
            pltpu.VMEM((NQ, H, LANES // 2, TQ), jnp.uint32),
            pltpu.VMEM((NT_K, S, LANES), bf16),
            pltpu.VMEM((NRB, H, VROWS, RB), f32),
            pltpu.VMEM((D, 2 * LANES), bf16),
            pltpu.VMEM((2 * D, D), bf16),
            pltpu.VMEM((TQ, D), f32),
            pltpu.VMEM((D, TQ), f32),
            pltpu.VMEM((TQ, D), bf16),
            pltpu.SemaphoreType.DMA((TQ // OB,)),
        ] + [pltpu.VMEM((S, TQ), f32) for _ in range(NBUF)],
        compiler_params=pltpu.CompilerParams(
            dimension_semantics=("arbitrary",),
            vmem_limit_bytes=96 * 1024 * 1024,
        ),
    )(A_x.reshape(S, D), A_wqkv, A_wo, B_w_gate, B_w_up, B_w_down)
    return out.reshape(A_x.shape)
```
